```python
import os as _os
_os.environ.setdefault('JAX_PLATFORMS', 'cpu')
import jax
import jax.numpy as jnp

def _softmax(x, axis=-1):
    return jax.nn.softmax(x, axis=axis)

def _gelu(x):
    return jax.nn.gelu(x, approximate=True)

def _silu(x):
    return jax.nn.silu(x)

def _sigmoid(x):
    return jax.nn.sigmoid(x)

def _layernorm(x, axis=-1, eps=1e-05):
    m = jnp.mean(x, axis=axis, keepdims=True)
    v = jnp.var(x, axis=axis, keepdims=True)
    return (x - m) / jnp.sqrt(v + eps)

def _scatter_add(tgt, idx, src, axis=0):
    return tgt.at[idx].add(src)

def _segment_sum(src, seg, n):
    return jax.ops.segment_sum(src, seg, n)

class _Rng:

    def __init__(self, key):
        self._k = key

    def _next(self):
        self._k, sub = jax.random.split(self._k)
        return sub

    def normal(self, shape):
        return jax.random.normal(self._next(), shape, dtype=jnp.bfloat16)

    def randint(self, lo, hi, shape):
        return jax.random.randint(self._next(), shape, lo, hi, dtype=jnp.int32)

    def uniform(self, shape, lo=0.0, hi=1.0):
        return jax.random.uniform(self._next(), shape, jnp.bfloat16, lo, hi)

    def permutation(self, n):
        return jax.random.permutation(self._next(), n)
kernel_name = 'adaLN_cond__mha_block__geglu_ffn__prompt'

def setup_inputs():
    _rng = _Rng(jax.random.key(int.from_bytes(__import__("os").urandom(4), "little")))
    _w = lambda a: (lambda t: t.astype(jnp.bfloat16) if jnp.issubdtype(t.dtype, jnp.floating) else t)(jnp.asarray(a))

    def _A_setup():
        B, S, D, H = (1, 2048, 512, 32)
        return {'x': _w((lambda *s: _rng.normal(s) * 0.05)(B, S, D)), 'wqkv': _w((lambda *s: _rng.normal(s) * 0.05)(D, 3 * D)), 'wo': _w((lambda *s: _rng.normal(s) * 0.05)(D, D))}
    _A_in = _A_setup()

    def _B_setup():
        B, S, D, F = (1, 2048, 512, 1376)
        return {'x': _w((lambda *s: _rng.normal(s) * 0.05)(B, S, D)), 'w_gate': _w((lambda *s: _rng.normal(s) * 0.05)(D, F)), 'w_up': _w((lambda *s: _rng.normal(s) * 0.05)(D, F)), 'w_down': _w((lambda *s: _rng.normal(s) * 0.05)(F, D))}
    _B_in = _B_setup()
    return {'A_x': _A_in['x'], 'A_wqkv': _A_in['wqkv'], 'A_wo': _A_in['wo'], 'B_x': _B_in['x'], 'B_w_gate': _B_in['w_gate'], 'B_w_up': _B_in['w_up'], 'B_w_down': _B_in['w_down'], 'c': _w((lambda *s: _rng.normal(s) * 0.05)(1, 512) * 8.0), 'w_mod': _w((lambda *s: _rng.normal(s) * 0.05)(512, 6 * 512) * 512 ** (-0.5) * 8.0)}

def reference(A_x, A_wqkv, A_wo, B_x, B_w_gate, B_w_up, B_w_down, c, w_mod):

    def _A_ref(x, wqkv, wo):
        B, S, D = x.shape
        H = 32
        Dh = D // H
        qkv = (lambda x, *d: x.transpose(*d))((x @ wqkv).reshape(B, S, 3, H, Dh), 2, 0, 3, 1, 4)
        q, k, v = (qkv[0], qkv[1], qkv[2])
        scores = jnp.einsum('bhqd,bhkd->bhqk', q, k) * Dh ** (-0.5)
        p = _softmax(scores, axis=-1)
        o = jnp.einsum('bhqk,bhkd->bhqd', p, v)
        return (lambda x, *d: x.transpose(*d))(o, 0, 2, 1, 3).reshape(B, S, D) @ wo

    def _B_ref(x, w_gate, w_up, w_down):
        return _gelu(x @ w_gate) * (x @ w_up) @ w_down
    x = A_x
    mod = (_silu(c) @ w_mod).reshape(c.shape[0], 6, 1, -1)
    sa, ca, ga, sb, cb, gb = (mod[:, 0].copy(), mod[:, 1].copy(), mod[:, 2].copy(), mod[:, 3].copy(), mod[:, 4].copy(), mod[:, 5].copy())
    h = _layernorm(x, axis=-1) * (1 + ca) + sa
    x = x + ga * _A_ref(h, A_wqkv, A_wo)
    h = _layernorm(x, axis=-1) * (1 + cb) + sb
    x = x + gb * _B_ref(h, B_w_gate, B_w_up, B_w_down)
    return x
```

```python
import functools
import math

import jax
import jax.numpy as jnp
from jax import lax
import jax.experimental.pallas as pl
import jax.experimental.pallas.tpu as pltpu

F32, BF16, I32, I16, I8 = jnp.float32, jnp.bfloat16, jnp.int32, jnp.int16, jnp.int8

H = 32
LANES = 128
LN_EPS = 1e-5
MAGIC = 12582912.0
QMAX, KMAX = 254.0, 381.0
CQ, CK = 24.0, 24.0
LOGIT_LIMIT = 64.0
TINY = 1e-30

NT = (((1,), (1,)), ((), ()))


def _dot(a, b):
    return jnp.dot(a, b, preferred_element_type=F32)


def _dot_nt(a, b):
    return lax.dot_general(a, b, NT, preferred_element_type=F32)


def _norm_mod(x, scale1, shift):
    m = jnp.mean(x, axis=-1, keepdims=True)
    xc = x - m
    v = jnp.mean(xc * xc, axis=-1, keepdims=True)
    return xc * lax.rsqrt(v + LN_EPS) * scale1 + shift


def _gelu(x):
    c0 = math.sqrt(2.0 / math.pi)
    inner = x * (c0 + (c0 * 0.044715) * (x * x))
    return (0.5 * x) * (1.0 + jnp.tanh(inner))


def _limb(v):
    return lax.bitcast_convert_type(v + MAGIC, I32)


def _kernel(x_hbm, wqkv_hbm, wo_hbm, wg_hbm, wu_hbm, wd_hbm, c_hbm, wmod_hbm, out_hbm,
            x_v, wqkv_v, wo_v, wg_v, wu_v, wd_v, c_v, wmod_v, out_v,
            wt_v, h_v, kt_v, mid_v, inv_v, rad_v, kenc_v, qenc_v, qs_v, vt_v, ot_v, x1_v, mod_v,
            sem, osem, *, cfg):
    S, D = x_v.shape
    DH = D // H
    Fdim = wg_v.shape[0]
    TB = cfg["TB"]
    NB = S // TB
    scale = DH ** -0.5 * math.log2(math.e)

    def cp(src, dst, i):
        return pltpu.make_async_copy(src, dst, sem.at[i])

    def cols(a, b):
        return (slice(None), slice(a, b))

    cp_c = cp(c_hbm, c_v, 0)
    cp_mod_a = cp(wmod_hbm.at[cols(0, 2 * D)], wmod_v.at[cols(0, 2 * D)], 1)
    cp_wk = cp(wqkv_hbm.at[cols(D, 2 * D)], wqkv_v.at[cols(D, 2 * D)], 2)
    cp_wq = cp(wqkv_hbm.at[cols(0, D)], wqkv_v.at[cols(0, D)], 3)
    cp_wv = cp(wqkv_hbm.at[cols(2 * D, 3 * D)], wqkv_v.at[cols(2 * D, 3 * D)], 4)
    cp_mod_b = cp(wmod_hbm.at[cols(2 * D, 6 * D)], wmod_v.at[cols(2 * D, 6 * D)], 5)
    cp_wo = cp(wo_hbm, wo_v, 6)
    cp_wg = cp(wg_hbm, wg_v, 7)
    cp_wu = cp(wu_hbm, wu_v, 8)
    cp_wd = cp(wd_hbm, wd_v, 9)
    cp_x = [cp(x_hbm.at[pl.ds(b * TB, TB)], x_v.at[pl.ds(b * TB, TB)], 10 + b) for b in range(NB)]

    cp_c.start()
    cp_wk.start()
    cp_mod_a.start()
    cp_x[0].start()

    cp_c.wait()
    cv = c_v[...].astype(F32)
    sc = jnp.broadcast_to(cv * jax.nn.sigmoid(cv), (16, D)).astype(BF16)
    cp_wk.wait()
    for b in range(1, NB):
        cp_x[b].start()
    wt_v[D:2 * D, :] = wqkv_v[:, D:2 * D].T
    cp_mod_a.wait()
    cp_wv.start()
    cp_wq.start()
    mod_a = _dot(sc, wmod_v[:, 0:2 * D])
    sa = mod_a[0:1, 0:D]
    ca1 = 1.0 + mod_a[0:1, D:2 * D]

    hi = lo = None
    for b in range(NB):
        rows = slice(b * TB, (b + 1) * TB)
        cp_x[b].wait()
        h = _norm_mod(x_v[rows, :].astype(F32), ca1, sa).astype(BF16)
        h_v[rows, :] = h
        kt = _dot_nt(wt_v[D:2 * D, :], h)
        kt_v[:, rows] = kt
        for j in range(TB // LANES):
            t = kt[:, j * LANES:(j + 1) * LANES]
            hi = t if hi is None else jnp.maximum(hi, t)
            lo = t if lo is None else jnp.minimum(lo, t)
    cp_wv.wait()
    cp_wq.wait()
    for d in (cp_wo, cp_mod_b, cp_wg, cp_wu, cp_wd):
        d.start()
    wt_v[2 * D:3 * D, :] = wqkv_v[:, 2 * D:3 * D].T
    wt_v[0:D, :] = wqkv_v[:, 0:D].T
    hi = jnp.max(hi, axis=1, keepdims=True)
    lo = jnp.min(lo, axis=1, keepdims=True)
    rad = jnp.maximum(0.5 * hi - 0.5 * lo, TINY)
    mid_v[...] = jnp.broadcast_to(0.5 * hi + 0.5 * lo, (D, LANES))
    inv_v[...] = jnp.broadcast_to(KMAX / rad, (D, LANES))
    rad_v[...] = jnp.broadcast_to(rad * scale, (D, LANES))

    def rep(a):
        return jnp.concatenate([a] * (TB // LANES), axis=1)

    def phase2(b, bound):
        tok = pl.ds(pl.multiple_of(b * TB, TB), TB)
        h = h_v[tok, :]
        qt = _dot_nt(wt_v[0:D, :], h)
        vt_v[:, tok] = _dot_nt(wt_v[2 * D:3 * D, :], h).astype(BF16)
        for hd in range(H):
            r = slice(hd * DH, (hd + 1) * DH)
            y = (kt_v[r, tok] - rep(mid_v[r, :])) * rep(inv_v[r, :])
            yi = (y + MAGIC) - MAGIC
            u = yi * (1.0 / 3.0)
            b1 = _limb(u).astype(I16)
            b2 = _limb(u + 1.0 / 3.0).astype(I16)
            b3 = _limb(u - 1.0 / 3.0).astype(I16)
            be = _limb((y - yi) * CQ).astype(I16)
            bc = _limb(y * (1.0 / CK)).astype(I16)
            kenc = jnp.concatenate([b1, b1, b2, b2, b3, b3, be, bc], axis=0)
            kenc_v[hd, tok, :] = kenc.T.astype(I8)
        for hd in range(H):
            r = slice(hd * DH, (hd + 1) * DH)
            qp = qt[r, :] * rep(rad_v[r, :])
            aq = jnp.abs(qp)
            amax = jnp.maximum(jnp.max(aq, axis=0, keepdims=True), TINY)
            bound = jnp.maximum(bound, jnp.sum(aq, axis=0, keepdims=True))
            xq = qp * (QMAX / amax)
            xi = (xq + MAGIC) - MAGIC
            u = xi * 0.5
            a1 = _limb(u + 0.25)
            a2 = _limb(u - 0.25)
            ac = _limb(xi * (1.0 / CQ))
            ae = _limb((xq - xi) * CK)
            qenc_v[hd, :, tok] = jnp.concatenate([a1, a2, ac, ae], axis=0).astype(I8)
            qs_v[hd, :, tok] = jnp.broadcast_to(amax * (1.0 / (QMAX * KMAX)), (8, TB))
        return bound

    bound = jnp.zeros((1, TB), F32)
    if cfg["unroll2"]:
        for b in range(NB):
            bound = phase2(b, bound)
    else:
        bound = lax.fori_loop(0, NB, phase2, bound)
    fast = jnp.max(jnp.where(bound <= cfg.get("limit", LOGIT_LIMIT), 0.0, 1.0)) == 0.0

    TQ, TK, HU, LAG, G = cfg["TQ"], LANES, cfg["HU"], cfg["LAG"], cfg["G"]
    NC = S // TK

    @pl.when(fast)
    def _():
        def body(i, carry):
            h0 = (i % (H // HU)) * HU
            tq = pl.ds(pl.multiple_of((i // (H // HU)) * TQ, TQ), TQ)
            n = HU * NC // G
            ps, acc, den = {}, {}, {}
            for t in range(n + LAG):
                if t < n:
                    u, c = divmod(t, NC // G)
                    qe = qenc_v[h0 + u, :, tq]
                    qe = jnp.concatenate([qe[0:32], qe[0:32], qe], axis=0)
                    r = jnp.dot(kenc_v[h0 + u, c * TK * G:(c + 1) * TK * G, :], qe, preferred_element_type=I32)
                    p = jnp.exp2(r.astype(F32).reshape(G * TK // 8, 8, TQ) * qs_v[h0 + u, :, tq][None])
                    part = jnp.sum(p, axis=0)
                    den[u] = part if c == 0 else den[u] + part
                    ps[t] = p.reshape(G * TK, TQ).astype(BF16)
                if t >= LAG:
                    u, c = divmod(t - LAG, NC // G)
                    hr = pl.ds(pl.multiple_of((h0 + u) * DH, DH), DH)
                    p = ps.pop(t - LAG)
                    for g in range(G):
                        k0 = (c * G + g) * TK
                        o = _dot(vt_v[hr, k0:k0 + TK], p[g * TK:(g + 1) * TK])
                        acc[u] = o if (c == 0 and g == 0) else acc[u] + o
                    if c == NC // G - 1:
                        l = jnp.sum(den.pop(u), axis=0, keepdims=True)
                        ot_v[hr, tq] = (acc.pop(u) * (1.0 / l)).astype(BF16)
            return carry
        lax.fori_loop(0, (S // TQ) * (H // HU), body, 0)

    @pl.when(jnp.logical_not(fast))
    def _():
        def body(i, carry):
            g = i // NB
            tq = pl.ds(pl.multiple_of((i % NB) * TB, TB), TB)
            gr = pl.multiple_of(g * LANES, LANES)
            k = _dot_nt(h_v[...], wt_v[pl.ds(D + gr, LANES), :]).astype(BF16)
            qt = _dot_nt(wt_v[pl.ds(gr, LANES), :], h_v[tq, :])
            head = lax.broadcasted_iota(I32, (LANES, TB), 0) // DH

            def one(j, carry):
                s = _dot(k, jnp.where(head == j, qt, 0.0).astype(BF16)) * scale
                p = jnp.exp2(s - jnp.max(s, axis=0, keepdims=True))
                l = jnp.sum(p, axis=0, keepdims=True)
                hr = pl.ds(pl.multiple_of(gr + j * DH, DH), DH)
                ot_v[hr, tq] = (_dot(vt_v[hr, :], p.astype(BF16)) * (1.0 / l)).astype(BF16)
                return carry
            return lax.fori_loop(0, LANES // DH, one, carry)
        lax.fori_loop(0, (D // LANES) * NB, body, 0)

    for d in (cp_wo, cp_mod_b, cp_wg, cp_wu, cp_wd):
        d.wait()
    mod_b = _dot(sc, wmod_v[:, 2 * D:6 * D])
    ga = mod_b[0:1, 0:D]
    sb = mod_b[0:1, D:2 * D]
    cb1 = 1.0 + mod_b[0:1, 2 * D:3 * D]
    mod_v[...] = mod_b[0:8, 3 * D:4 * D]
    for b in range(NB):
        rows = slice(b * TB, (b + 1) * TB)
        x1 = x_v[rows, :].astype(F32) + ga * _dot(ot_v[:, rows].T, wo_v[...])
        x1_v[rows, :] = x1
        h_v[rows, :] = _norm_mod(x1, cb1, sb).astype(BF16)

    TF, FC = cfg["TF"], cfg["FC"]
    chunks = [(f, min(f + FC, Fdim)) for f in range(0, Fdim, FC)]

    def out_copy(b):
        rows = pl.ds(pl.multiple_of(b * TF, TF), TF)
        return pltpu.make_async_copy(out_v.at[rows], out_hbm.at[rows], osem.at[b])

    def ffn(b, carry):
        rows = pl.ds(pl.multiple_of(b * TF, TF), TF)
        h = h_v[rows, :]
        acts, y = {}, None
        for t in range(len(chunks) + 1):
            if t < len(chunks):
                f0, f1 = chunks[t]
                acts[t] = (_gelu(_dot_nt(h, wg_v[f0:f1, :])) * _dot_nt(h, wu_v[f0:f1, :])).astype(BF16)
            if t >= 1:
                f0, f1 = chunks[t - 1]
                part = _dot(acts.pop(t - 1), wd_v[f0:f1, :])
                y = part if y is None else y + part
        out_v[rows, :] = (x1_v[rows, :] + mod_v[0:1, :] * y).astype(out_v.dtype)
        out_copy(b).start()
        return carry

    if cfg["unroll5"]:
        for b in range(S // TF):
            ffn(b, 0)
    else:
        lax.fori_loop(0, S // TF, ffn, 0)
    for b in range(S // TF):
        out_copy(b).wait()


DEFAULT = dict(TB=512, unroll2=False, TQ=512, HU=4, LAG=3, G=1, TF=512, FC=512, unroll5=False)


def build(**kw):
    cfg = dict(DEFAULT, **kw)

    def fn(A_x, A_wqkv, A_wo, B_x, B_w_gate, B_w_up, B_w_down, c, w_mod):
        del B_x
        B, S, D = A_x.shape
        Fdim = B_w_gate.shape[1]
        V = pltpu.VMEM
        scratch = [
            V((S, D), BF16), V((D, 3 * D), BF16), V((D, D), BF16), V((Fdim, D), BF16), V((Fdim, D), BF16),
            V((Fdim, D), BF16), V((1, D), BF16), V((D, 6 * D), BF16), V((S, D), BF16),
            V((3 * D, D), BF16), V((S, D), BF16), V((D, S), F32), V((D, LANES), F32), V((D, LANES), F32),
            V((D, LANES), F32), V((H, S, LANES), I8), V((H, 64, S), I8), V((H, 8, S), F32), V((D, S), BF16),
            V((D, S), BF16), V((S, D), F32), V((8, D), F32),
            pltpu.SemaphoreType.DMA((10 + S // cfg["TB"],)), pltpu.SemaphoreType.DMA((S // cfg["TF"],)),
        ]
        out = pl.pallas_call(
            functools.partial(_kernel, cfg=cfg),
            out_shape=jax.ShapeDtypeStruct((S, D), A_x.dtype),
            in_specs=[pl.BlockSpec(memory_space=pltpu.HBM)] * 8,
            out_specs=pl.BlockSpec(memory_space=pltpu.HBM),
            scratch_shapes=scratch,
            compiler_params=pltpu.CompilerParams(vmem_limit_bytes=100 * 2**20, flags=cfg.get("flags")),
            name="blk",
        )(A_x.reshape(S, D), A_wqkv, A_wo, B_w_gate.T, B_w_up.T, B_w_down, c, w_mod)
        return out.reshape(B, S, D)
    return jax.jit(fn)


pallas_adaLN_cond__mha_block__geglu_ffn__prompt_kernel = build(**{'HU':8})
```

```python
import functools
import math

import jax
import jax.numpy as jnp
from jax import lax
import jax.experimental.pallas as pl
import jax.experimental.pallas.tpu as pltpu

F32, BF16, I32, I16, I8 = jnp.float32, jnp.bfloat16, jnp.int32, jnp.int16, jnp.int8

H = 32
L = 128
LN_EPS = 1e-5

MAGIC = 1.5 * 2.0 ** 23
QMAX, KMAX = 253.0, 376.0
FRAC = 4
TINY = 1e-30
TERM_LIMIT = 24.0
DEN_LO, DEN_HI = 2.0 ** -40, 2.0 ** 40

X_PIECES = ((2, 1), (4, 3), (9, 8), (16, 16))


def _dot(a, b):
    return jnp.dot(a, b, preferred_element_type=F32)


def _dot_nt(a, b):
    return lax.dot_general(a, b, (((1,), (1,)), ((), ())), preferred_element_type=F32)


def _cat(parts, axis):
    return jnp.concatenate(parts, axis=axis)


def _ds(start, size):
    return pl.ds(start if isinstance(start, int) else pl.multiple_of(start, size), size)


def _pack(v):
    return pltpu.bitcast(v.astype(BF16), I32)


def _unpack(v):
    return pltpu.bitcast(v, BF16)


def _normalize(x):
    xc = x - jnp.mean(x, axis=-1, keepdims=True)
    return xc * lax.rsqrt(jnp.mean(xc * xc, axis=-1, keepdims=True) + LN_EPS)


def _gelu(x):
    c0 = math.sqrt(2.0 / math.pi)
    return (0.5 * x) * (1.0 + jnp.tanh(x * (c0 + (c0 * 0.044715) * (x * x))))


def _fixed(v, shift, bias=0.0):
    return lax.bitcast_convert_type(v + (MAGIC + bias) * 2.0 ** -shift, I32)


def _lhs7(a11, a12, a21, a22):
    return [a11 + a22, a21 + a22, a11, a22, a11 + a12, a21 - a11, a12 - a22]


def _rhs7(b11, b12, b21, b22):
    return [b11 + b22, b11, b12 - b22, b21 - b11, b22, b11 + b12, b21 + b22]


def _strassen(prod):
    c11 = c22 = prod(0)
    c22 = c22 + prod(5)
    c11 = c11 + prod(6)
    m = prod(1)
    c21, c22 = m, c22 - m
    m = prod(3)
    c21, c11 = c21 + m, c11 + m
    m = prod(2)
    c12, c22 = m, c22 + m
    m = prod(4)
    c12, c11 = c12 + m, c11 - m
    return c11, c12, c21, c22


def _block_kernel(x_hbm, wqkv_hbm, wo_hbm, wg_hbm, wu_hbm, wd_hbm, c_hbm, wmod_hbm, out_hbm,
                  x_v, wqkv_v, wo_v, wg_v, wu_v, wd_v, c_v, wmod_v, out_v,
                  mod_v, wt_v, h_v, kq_v, kstat_v, qscale_v, limb_v, vt_v, p_v, acc_v, ot_v,
                  kb_v, sa_v, sb_v, wo7_v, wgu7_v, wd7_v, x1_v, h7_v, yt_v, sem, out_sem, *, cfg):
    S, D = x_v.shape
    F = wd_v.shape[0]
    DH, HD = D // H, D // 2
    FH = (F // (2 * L)) * L
    FR = (F - 2 * FH) // 2
    TP = 2 * L
    NT, NP = S // L, S // TP
    logit_scale = DH ** -0.5 * math.log2(math.e)
    X_PIECES = cfg["regions"]

    def cols(a, b):
        return (slice(None), slice(a * D, b * D))

    x_rows = [slice(a * L, b * L) for a, (b, _) in zip([0] + [n for n, _ in X_PIECES], X_PIECES)]
    jobs = [("c", c_hbm, c_v),
            ("wk", wqkv_hbm.at[cols(1, 2)], wqkv_v.at[cols(1, 2)]),
            ("x0", x_hbm.at[x_rows[0]], x_v.at[x_rows[0]]),
            ("mod_a", wmod_hbm.at[cols(0, 2)], wmod_v.at[cols(0, 2)])]
    jobs += [("x%d" % i, x_hbm.at[r], x_v.at[r]) for i, r in enumerate(x_rows) if i]
    jobs += [("wq", wqkv_hbm.at[cols(0, 1)], wqkv_v.at[cols(0, 1)]),
             ("wv", wqkv_hbm.at[cols(2, 3)], wqkv_v.at[cols(2, 3)]),
             ("mod_b", wmod_hbm.at[cols(2, 6)], wmod_v.at[cols(2, 6)]),
             ("wo", wo_hbm, wo_v), ("wg", wg_hbm, wg_v), ("wu", wu_hbm, wu_v), ("wd", wd_hbm, wd_v)]
    dma = {name: pltpu.make_async_copy(src, dst, sem.at[i]) for i, (name, src, dst) in enumerate(jobs)}
    for copy in dma.values():
        copy.start()

    def wait(*names):
        for name in names:
            dma[name].wait()

    def transpose_weight(w):
        wt_v[w] = _pack(wqkv_v[:, w * D:(w + 1) * D].T)

    def project(w, t):
        return _dot_nt(_unpack(wt_v[w]), h_v[_ds(t * L, L), :])

    wait("c", "wk")
    cv = c_v[...].astype(F32)
    silu_c = jnp.broadcast_to(cv * jax.nn.sigmoid(cv), (16, D)).astype(BF16)
    transpose_weight(1)
    wait("x0")
    xn = _normalize(x_v[x_rows[0], :].astype(F32))
    wait("mod_a")
    mod_a = _dot(silu_c, wmod_v[:, 0:2 * D])
    sa, ca1 = mod_a[0:1, 0:D], 1.0 + mod_a[0:1, D:2 * D]

    hi = lo = None
    n0 = k0 = 0
    for i, (n1, k1) in enumerate(X_PIECES):
        if i:
            wait("x%d" % i)
        if i == len(X_PIECES) - 1:
            wait("wq", "wv")
        for t in range(n0, n1):
            rows = slice(t * L, (t + 1) * L)
            xt = _normalize(x_v[rows, :].astype(F32)) if i else xn[rows]
            h_v[rows, :] = (xt * ca1 + sa).astype(BF16)
        for t in range(k0, k1):
            kt = project(1, t)
            kq_v[0:D, t * L:(t + 1) * L] = kt
            hi = kt if hi is None else jnp.maximum(hi, kt)
            lo = kt if lo is None else jnp.minimum(lo, kt)
        n0, k0 = n1, k1
    transpose_weight(0)
    transpose_weight(2)
    hi = jnp.max(hi, axis=1, keepdims=True)
    lo = jnp.min(lo, axis=1, keepdims=True)
    mid = 0.5 * hi + 0.5 * lo
    rad = jnp.maximum(jnp.maximum(hi - mid, mid - lo), TINY)
    kstat_v[0] = jnp.broadcast_to(mid, (D, L))
    kstat_v[1] = jnp.broadcast_to(KMAX / rad, (D, L))
    kstat_v[2] = jnp.broadcast_to(rad * logit_scale, (D, L))

    def q_steps(t, top):
        tok = _ds(t * L, L)
        q = project(0, t) * kstat_v[2]
        a = jnp.abs(q)
        sub = lax.broadcasted_iota(I32, (8, L), 0)
        for g in range(D // L):
            kq_v[D + g * L:D + g * L + 64, tok] = q[g * L:g * L + 64]
            yield
            kq_v[D + g * L + 64:D + (g + 1) * L, tok] = q[g * L + 64:(g + 1) * L]
            m = [jnp.maximum(a[DH * j:DH * j + 8], a[DH * j + 8:DH * j + 16]) for j in range(8 * g, 8 * g + 8)]
            for w in (4, 2, 1):
                m = [jnp.where((sub & w) == 0,
                               jnp.maximum(m[j], pltpu.roll(m[j], 8 - w, 0)),
                               jnp.maximum(m[j + w], pltpu.roll(m[j + w], w, 0))) for j in range(w)]
            amax = jnp.maximum(m[0], TINY)
            top[0] = jnp.maximum(top[0], amax)
            yield
            qscale_v[H + 8 * g:H + 8 * g + 8, tok] = QMAX / amax
            qscale_v[8 * g:8 * g + 8, tok] = amax * (1.0 / (QMAX * KMAX))

    def v_steps(t):
        vt = project(2, t)
        for r in range(0, D, 64):
            vt_v[t, r // 2:r // 2 + 32, :] = _pack(vt[r:r + 64])
            yield

    def limbs(hd, p):
        r = slice(hd * DH, (hd + 1) * DH)
        tok = _ds(p * TP, TP)
        y = (kq_v[r, tok] - _cat([kstat_v[0, r]] * 2, 1)) * _cat([kstat_v[1, r]] * 2, 1)
        z = _fixed(y, FRAC, 2.0 ** (FRAC - 1))
        b1 = lax.bitcast_convert_type(y * (-1.0 / 3.0) - MAGIC, I32)
        b3 = ((z >> FRAC) - b1 - b1).astype(I16)
        b1 = b1.astype(I16)
        be = (z & (2 ** FRAC - 1)).astype(I16)
        bc = _fixed(y, -FRAC).astype(I16)
        kl = _cat([b1, b1, b1, b1, b3, b3, be, bc], 0).T.astype(I8)
        for j in range(TP // 32):
            limb_v[hd, _ds(p * TP + (j // 4) * L + (3 - j % 4) * 32, 32), :] = kl[32 * j:32 * j + 32]
        x = kq_v[D + hd * DH:D + (hd + 1) * DH, tok] * qscale_v[H + hd:H + hd + 1, tok]
        z = _fixed(x, FRAC, 2.0 ** (FRAC - 1))
        a1 = _fixed(x, -1)
        a2 = (z >> FRAC) - a1
        ac = _fixed(x, -FRAC)
        ae = (z & (2 ** FRAC - 1)) - 2 ** (FRAC - 1)
        ql = _cat([a1, a2, ac, ae], 0).astype(I8)
        for i in range(2):
            limb_v[hd, _ds(S + p * L + 64 * i, 64), :] = ql[:, i * L:(i + 1) * L]

    def phase2(p, top, last=False):
        top = [top]
        gens = [] if last else [q_steps(2 * p + 2 + j, top) for j in range(2)]
        gens += [v_steps(2 * p + j) for j in range(2)]
        lead = done = cfg["lead"]
        for hd in range(lead):
            limbs(hd, p)
        step = 0
        for gen in gens:
            for _ in gen:
                step += 1
                upto = min(H, lead + ((H - lead) * step) // (8 * len(gens) - cfg["s1"]))
                for hd in range(done, upto):
                    limbs(hd, p)
                done = upto
        return top[0]

    top = [jnp.zeros((8, L), F32)]
    for t in range(2):
        for _ in q_steps(t, top):
            pass
    top = lax.fori_loop(0, NP - 1, phase2, top[0], unroll=cfg["U2"])
    wait("mod_b", "wo", "wg", "wu", "wd")
    too_wide = jnp.max(jnp.where(top <= cfg.get("limit", TERM_LIMIT), 0.0, 1.0))
    phase2(NP - 1, top, last=True)
    mod_v[...] = _dot(silu_c, wmod_v[:, 2 * D:6 * D])[0:8]
    p_v[...] = jnp.zeros(p_v.shape, p_v.dtype)
    acc_v[...] = jnp.ones(acc_v.shape, acc_v.dtype)

    TQ, HU, G = 4 * L, 8, 2
    NI = (S // TQ) * (H // HU)

    def prepare_weights(i):
        for q in range(-(-(FH + FR) // (16 * NI))):
            r = jnp.minimum((q * NI + i) * 16, FH + FR - 16)
            r1 = jnp.where(r < FH, r, r + FH)
            r2 = jnp.where(r < FH, r + FH, r + FH + FR)
            for w, src in enumerate((wg_v, wu_v)):
                a1, a2 = src[_ds(r1, 16), :].astype(F32), src[_ds(r2, 16), :].astype(F32)
                for n, op in enumerate(_lhs7(a1[:, :HD], a1[:, HD:], a2[:, :HD], a2[:, HD:])):
                    for j in range(HD // L):
                        wgu7_v[w, n, j, _ds(r, 16), :] = op[:, j * L:(j + 1) * L].astype(BF16)
        rows = HD // NI
        b1, b2 = wo_v[_ds(i * rows, rows), :].astype(F32), wo_v[_ds(HD + i * rows, rows), :].astype(F32)
        for n, op in enumerate(_rhs7(b1[:, :HD], b1[:, HD:], b2[:, :HD], b2[:, HD:])):
            for j in range(HD // L):
                wo7_v[n, j, _ds(i * rows, rows), :] = op[:, j * L:(j + 1) * L].astype(BF16)

    def pv(hd, c, p):
        return _dot(_unpack(vt_v[c, _ds(hd * (DH // 2), DH // 2), :]), p)

    def store_o(o, hd, qb):
        for j in range(TQ // L):
            ot_v[qb * (TQ // L) + j, _ds(hd * DH, DH), :] = o[:, j * L:(j + 1) * L]

    def finalize(acc, den, hd, qb, bad):
        l = jnp.sum(den, axis=0, keepdims=True)
        store_o(acc * pltpu.reciprocal(l, full_range=False), hd, qb)
        return jnp.where((l >= DEN_LO) & (l <= cfg.get("hi", DEN_HI)), bad, 1.0)

    def attend(i, bad):
        h0, qb = (i % (H // HU)) * HU, i // (H // HU)
        ip = jnp.maximum(i - 1, 0)
        scales = qscale_v[_ds(h0, HU), _ds(qb * TQ, TQ)]
        prev = ((ip % (H // HU)) * HU + HU - 1, ip // (H // HU), NT - G, [_unpack(p_v[a]) for a in range(G)])
        acc, den = acc_v[0:DH], acc_v[DH:DH + 8]
        for u in range(HU):
            ql = _cat([limb_v[h0 + u, _ds(S + qb * (TQ // 2) + 64 * j, 64), :] for j in range(TQ // L)], 1)
            ql = _cat([ql[0:32], ql[0:32], ql], 0)
            scale = jnp.broadcast_to(scales[u:u + 1], (8, TQ))
            d = None
            for c in range(0, NT, G):
                s = jnp.dot(limb_v[h0 + u, c * L:(c + G) * L, :], ql, preferred_element_type=I32)
                e = []
                for j in range(G * L // 8):
                    e.append(jnp.exp2(s[8 * j:8 * j + 8].astype(F32) * scale))
                    d = e[-1] if d is None else d + e[-1]
                p = [_cat([e[16 * a + 4 * (3 - j // 4) + j % 4] for j in range(16)], 0).astype(BF16)
                     for a in range(G)]
                hd, pqb, pc, pp = prev
                o = pv(hd, pc, pp[0]) + pv(hd, pc + 1, pp[1])
                acc = o if acc is None else acc + o
                if pc == NT - G:
                    bad = finalize(acc, den, hd, pqb, bad)
                    acc = None
                prev = (h0 + u, qb, c, p)
            den = d
        for a in range(G):
            p_v[a] = _pack(prev[3][a])
        acc_v[0:DH], acc_v[DH:DH + 8] = acc, den
        prepare_weights(i)
        return bad

    bad = lax.fori_loop(0, jnp.where(too_wide == 0.0, NI, 0), attend, jnp.zeros((1, TQ), F32))
    acc = acc_v[0:DH] + pv(H - 1, NT - 2, _unpack(p_v[0])) + pv(H - 1, NT - 1, _unpack(p_v[1]))
    bad = finalize(acc, acc_v[DH:DH + 8], H - 1, S // TQ - 1, bad)

    @pl.when(jnp.maximum(jnp.max(bad), too_wide) != 0.0)
    def _plain_attention():
        def setup(t, carry):
            k = _dot(h_v[_ds(t * L, L), :], wqkv_v[:, D:2 * D])
            for g in range(D // L):
                kb_v[g, _ds(t * L, L), :] = k[:, g * L:(g + 1) * L].astype(BF16)
            kq_v[D:2 * D, _ds(t * L, L)] = project(0, t)
            return carry

        def weights(i, carry):
            prepare_weights(i)
            return carry

        lax.fori_loop(0, NT, setup, 0)
        lax.fori_loop(0, NI, weights, 0)
        items = (S // TQ) * H
        head = lax.broadcasted_iota(I32, (L, TQ), 0) // DH

        def step(n, cur, nxt, row_max):
            nn = jnp.minimum(n + 1, items - 1)
            g = (nn % H) // (L // DH)
            q = kq_v[_ds(D + g * L, L), _ds((nn // H) * TQ, TQ)]
            q = jnp.where(head == nn % (L // DH), q, 0.0).astype(BF16)
            mx = acc = den = None
            for c in range(NT):
                s = _dot(kb_v[g, c * L:(c + 1) * L, :], q)
                nxt[c * L:(c + 1) * L, :] = s
                t = jnp.max(s.reshape(L // 8, 8, TQ), axis=0)
                mx = t if mx is None else jnp.maximum(mx, t)
                if cur is not None:
                    e = jnp.exp2((cur[c * L:(c + 1) * L, :] - row_max) * logit_scale)
                    t = jnp.sum(e.reshape(L // 8, 8, TQ), axis=0)
                    o = pv(n % H, c, e.astype(BF16))
                    den, acc = (t, o) if c == 0 else (den + t, acc + o)
            if cur is not None:
                store_o(acc / jnp.sum(den, axis=0, keepdims=True), n % H, n // H)
            return jnp.max(mx, axis=0, keepdims=True)

        def two_steps(i, row_max):
            return step(2 * i + 1, sb_v, sa_v, step(2 * i, sa_v, sb_v, row_max))

        lax.fori_loop(0, items // 2, two_steps, step(-1, None, sa_v, None))

    ga, sb, cb1 = mod_v[0:1, 0:D], mod_v[0:1, D:2 * D], 1.0 + mod_v[0:1, 2 * D:3 * D]
    NR = 32

    def norm2(p, r0):
        h1, h2 = [_normalize(x1_v[_ds((2 * p + e) * L + r0, NR), :]) * cb1 + sb for e in range(2)]
        for n, op in enumerate(_rhs7(h1[:, :HD], h2[:, :HD], h1[:, HD:], h2[:, HD:])):
            for j in range(HD // L):
                h7_v[n, j, _ds(p * L + r0, NR), :] = op[:, j * L:(j + 1) * L].astype(BF16)

    for p in range(NP):
        o1, o2 = ot_v[2 * p], ot_v[2 * p + 1]
        lhs = _lhs7(o1[:HD], o1[HD:], o2[:HD], o2[HD:])
        blk = _strassen(lambda n: _dot(lhs[n].astype(BF16).T, _cat([wo7_v[n, j] for j in range(HD // L)], 1)))
        rows = slice(p * TP, (p + 1) * TP)
        x1_v[rows, :] = x_v[rows, :].astype(F32) + ga * _cat([_cat(blk[:2], 1), _cat(blk[2:], 1)], 0)
        if p == 1:
            for r0 in range(0, L, NR):
                norm2(0, r0)
        k = (p - 2) * L
        if 0 <= k < FH:
            for c0 in range(0, HD, L):
                w = [wd_v[r + k:r + k + L, c + c0:c + c0 + L].astype(F32) for c in (0, HD) for r in (0, FH)]
                for n, op in enumerate(_lhs7(*w)):
                    wd7_v[n, c0 // 2:(c0 + L) // 2, k:k + L] = _pack(op.astype(BF16).T)
    yt_v[...] = jnp.zeros(yt_v.shape, yt_v.dtype)

    chunks = [(FH, FH + FR)] + [(f, f + L) for f in range(0, FH, L)]

    def out_copy(p):
        rows = _ds(p * TP, TP)
        return pltpu.make_async_copy(out_v.at[rows], out_hbm.at[rows], out_sem.at[p])

    def finish(p):
        rows = _ds(p * TP, TP)
        y = _unpack(yt_v[...]).T.astype(F32)
        out_v[rows, :] = (x1_v[rows, :] + mod_v[0:1, 3 * D:4 * D] * y).astype(out_v.dtype)

    def ffn(p, carry):
        h7 = [_cat([h7_v[n, j, _ds(p * L, L), :] for j in range(HD // L)], 1) for n in range(7)]
        wd_rest = wd_v[2 * FH:, :].T
        finish(jnp.maximum(p - 1, 0))
        act7 = []
        for k, (f0, f1) in enumerate(chunks):
            def gate_up(n):
                w = _cat([_cat([wgu7_v[w, n, j, f0:f1, :] for j in range(HD // L)], 1) for w in range(2)], 0)
                m = _dot_nt(w, h7[n])
                if (k, n) == cfg["fl"]:
                    out_v[_ds(S + 16 * (p % 2), 16), 0:L] = m[-16:].astype(BF16)
                return m
            act = [_gelu(c[:f1 - f0]) * c[f1 - f0:] for c in _strassen(gate_up)]
            if f0 < FH:
                act7.append(_rhs7(*act))
            else:
                rest = _cat([_cat(act[:2], 1), _cat(act[2:], 1)], 0).astype(BF16)
        y = _cat([_dot(wd_rest[:HD], rest), _dot(wd_rest[HD:], rest)], 0)
        todo = list(range(0, L, NR))

        def down(n):
            m = _dot(_unpack(wd7_v[n]), _cat([a[n] for a in act7], 0).astype(BF16))
            if todo:
                x1_v[_ds(S + 8 * (p % 2), 8), 0:L] = m[0:8]
                norm2(jnp.minimum(p + 1, NP - 1), todo.pop(0))
            return m
        blk = _strassen(down)
        yt_v[...] = _pack(y + _cat([_cat(blk[:2], 1), _cat(blk[2:], 1)], 0))

        @pl.when(p > 0)
        def _():
            out_copy(p - 1).start()
        return carry

    lax.fori_loop(0, NP, ffn, 0)
    finish(NP - 1)
    out_copy(NP - 1).start()
    for p in range(NP):
        out_copy(p).wait()


DEFAULT = dict(regions=X_PIECES, lead=6, s1=6, U2=3, fl=(1, 6))


def build(interpret=False, **kw):
    cfg = dict(DEFAULT, **kw)

    def fn(A_x, A_wqkv, A_wo, B_x, B_w_gate, B_w_up, B_w_down, c, w_mod):
        del B_x
        B, S, D = A_x.shape
        F = B_w_gate.shape[1]
        vmem = pltpu.VMEM
        scratch = [
            vmem((S, D), BF16), vmem((D, 3 * D), BF16), vmem((D, D), BF16),
            vmem((F, D), BF16), vmem((F, D), BF16), vmem((F, D), BF16),
            vmem((1, D), BF16), vmem((D, 6 * D), BF16), vmem((S + 32, D), BF16),
            vmem((8, 4 * D), F32), vmem((3, D // 2, D), I32), vmem((S, D), BF16),
            vmem((2 * D, S), F32), vmem((3, D, L), F32), vmem((2 * H, S), F32),
            vmem((H, S + S // 2, L), I8), vmem((S // L, D // 2, L), I32),
            vmem((2, L // 2, 4 * L), I32), vmem((D // H + 8, 4 * L), F32),
            vmem((S // L, D, L), F32),
            vmem((D // L, S, L), BF16), vmem((S, 4 * L), F32), vmem((S, 4 * L), F32),
            vmem((7, 2, D // 2, L), BF16), vmem((2, 7, 2, F // 2, L), BF16),
            vmem((7, D // 4, F // (2 * L) * L), I32),
            vmem((S + 16, D), F32), vmem((7, 2, S // 2, L), BF16), vmem((D // 2, 2 * L), I32),
            pltpu.SemaphoreType.DMA((10 + len(cfg["regions"]),)), pltpu.SemaphoreType.DMA((S // (2 * L),)),
        ]
        out = pl.pallas_call(
            functools.partial(_block_kernel, cfg=cfg),
            out_shape=jax.ShapeDtypeStruct((S, D), A_x.dtype),
            in_specs=[pl.BlockSpec(memory_space=pltpu.HBM)] * 8,
            out_specs=pl.BlockSpec(memory_space=pltpu.HBM),
            scratch_shapes=scratch,
            compiler_params=pltpu.CompilerParams(vmem_limit_bytes=110 * 2 ** 20, flags=cfg.get("flags")),
            name="blk", interpret=interpret,
        )(A_x.reshape(S, D), A_wqkv, A_wo, B_w_gate.T, B_w_up.T, B_w_down, c, w_mod)
        return out.reshape(B, S, D)
    return jax.jit(fn)


pallas_adaLN_cond__mha_block__geglu_ffn__prompt_kernel = build(**{})
```

```python
import functools
import math

import jax
import jax.numpy as jnp
from jax import lax
import jax.experimental.pallas as pl
import jax.experimental.pallas.tpu as pltpu

F32, BF16, I32, I16, I8 = jnp.float32, jnp.bfloat16, jnp.int32, jnp.int16, jnp.int8

H = 32
L = 128
LN_EPS = 1e-5

MAGIC = 1.5 * 2.0 ** 23
QMAX, KMAX = 253.0, 376.0
FRAC = 4
TINY = 1e-30
TERM_LIMIT = 24.0
DEN_LO, DEN_HI = 2.0 ** -40, 2.0 ** 40
BALANCE = 4.0

X_PIECES = ((2, 1), (4, 3), (10, 9), (16, 16))


def _dot(a, b):
    return jnp.dot(a, b, preferred_element_type=F32)


def _dot_nt(a, b):
    return lax.dot_general(a, b, (((1,), (1,)), ((), ())), preferred_element_type=F32)


def _cat(parts, axis):
    return jnp.concatenate(parts, axis=axis)


def _ds(start, size):
    return pl.ds(start if isinstance(start, int) else pl.multiple_of(start, size), size)


def _pack(v):
    return pltpu.bitcast(v.astype(BF16), I32)


def _unpack(v):
    return pltpu.bitcast(v, BF16)


def _normalize(x):
    xc = x - jnp.mean(x, axis=-1, keepdims=True)
    return xc * lax.rsqrt(jnp.mean(xc * xc, axis=-1, keepdims=True) + LN_EPS)


def _gelu(x):
    c0 = math.sqrt(2.0 / math.pi)
    return (0.5 * x) * (1.0 + jnp.tanh(x * (c0 + (c0 * 0.044715) * (x * x))))


def _fixed(v, shift, bias=0.0):
    return lax.bitcast_convert_type(v + (MAGIC + bias) * 2.0 ** -shift, I32)


def _lhs7(a11, a12, a21, a22):
    return [a11 + a22, a21 + a22, a11, a22, a11 + a12, a21 - a11, a12 - a22]


def _rhs7(b11, b12, b21, b22):
    return [b11 + b22, b11, b12 - b22, b21 - b11, b22, b11 + b12, b21 + b22]


def _strassen(prod):
    c11 = c22 = prod(0)
    c22 = c22 + prod(5)
    c11 = c11 + prod(6)
    m = prod(1)
    c21, c22 = m, c22 - m
    m = prod(3)
    c21, c11 = c21 + m, c11 + m
    m = prod(2)
    c12, c22 = m, c22 + m
    m = prod(4)
    c12, c11 = c12 + m, c11 - m
    return c11, c12, c21, c22


def _block_kernel(x_hbm, wqkv_hbm, wo_hbm, wg_hbm, wu_hbm, wd_hbm, c_hbm, wmod_hbm, out_hbm,
                  x_v, wqkv_v, wo_v, wf_v, c_v, wmod_v, out_v,
                  mod_v, wt_v, h_v, kq_v, kstat_v, qscale_v, limb_v, vt_v, p_v, acc_v, ot_v,
                  kb_v, sa_v, sb_v, wgu7_v, wd7_v, x1_v, h7_v, yt_v, colsq_v, sem, out_sem):
    S, D = x_v.shape
    F = wd_hbm.shape[0]
    DH, HD = D // H, D // 2
    FH = (F // (2 * L)) * L
    FR = (F - 2 * FH) // 2
    TP = 2 * L
    NT, NP = S // L, S // TP
    logit_scale = DH ** -0.5 * math.log2(math.e)

    def cols(a, b):
        return (slice(None), slice(a * D, b * D))

    x_rows = [slice(a * L, b * L) for a, (b, _) in zip([0] + [n for n, _ in X_PIECES], X_PIECES)]
    last_x = "x%d" % (len(x_rows) - 1)
    groups = {"wk": [(c_hbm, c_v), (wqkv_hbm.at[cols(1, 2)], wqkv_v.at[cols(1, 2)])],
              "x0": [(x_hbm.at[x_rows[0]], x_v.at[x_rows[0]])],
              "mod": [(wmod_hbm.at[cols(0, 2)], wmod_v.at[cols(0, 2)])]}
    for i in range(1, len(x_rows)):
        groups["x%d" % i] = [(x_hbm.at[x_rows[i]], x_v.at[x_rows[i]])]
    groups[last_x] += [(wqkv_hbm.at[cols(w, w + 1)], wqkv_v.at[cols(w, w + 1)]) for w in (0, 2)]
    groups["rest"] = [(wmod_hbm.at[cols(2, 6)], wmod_v.at[cols(2, 6)]), (wo_hbm, wo_v)]
    groups["rest"] += [(src, wf_v.at[w, 0:F]) for w, src in enumerate((wg_hbm, wu_hbm, wd_hbm))]
    dma = {name: [pltpu.make_async_copy(src, dst, sem.at[i]) for src, dst in group]
           for i, (name, group) in enumerate(groups.items())}
    for group in dma.values():
        for copy in group:
            copy.start()

    def wait(name):
        for copy in dma[name]:
            copy.wait()

    def transpose_weight(w):
        wt_v[w] = _pack(wqkv_v[:, w * D:(w + 1) * D].T)

    def project(w, t):
        return _dot_nt(_unpack(wt_v[w]), h_v[_ds(t * L, L), :])

    wait("wk")
    cv = c_v[...].astype(F32)
    silu_c = jnp.broadcast_to(cv * jax.nn.sigmoid(cv), (16, D)).astype(BF16)
    transpose_weight(1)
    wait("x0")
    xn = _normalize(x_v[x_rows[0], :].astype(F32))
    wait("mod")
    mod_a = _dot(silu_c, wmod_v[:, 0:2 * D])
    sa, ca1 = mod_a[0:1, 0:D], 1.0 + mod_a[0:1, D:2 * D]

    hi = lo = None
    n0 = k0 = 0
    for i, (n1, k1) in enumerate(X_PIECES):
        if i:
            wait("x%d" % i)
        for t in range(n0, n1):
            rows = slice(t * L, (t + 1) * L)
            xt = _normalize(x_v[rows, :].astype(F32)) if i else xn[rows]
            h_v[rows, :] = (xt * ca1 + sa).astype(BF16)
        for t in range(k0, k1):
            kt = project(1, t)
            kq_v[0:D, t * L:(t + 1) * L] = kt
            hi = kt if hi is None else jnp.maximum(hi, kt)
            lo = kt if lo is None else jnp.minimum(lo, kt)
        n0, k0 = n1, k1
    transpose_weight(0)
    transpose_weight(2)
    hi = jnp.max(hi, axis=1, keepdims=True)
    lo = jnp.min(lo, axis=1, keepdims=True)
    mid = 0.5 * hi + 0.5 * lo
    rad = jnp.maximum(jnp.maximum(hi - mid, mid - lo), TINY)
    kstat_v[0] = jnp.broadcast_to(mid, (D, L))
    kstat_v[1] = jnp.broadcast_to(KMAX / rad, (D, L))
    kstat_v[2] = jnp.broadcast_to(rad * logit_scale, (D, L))

    def q_steps(t, top):
        tok = _ds(t * L, L)
        q = project(0, t) * kstat_v[2]
        a = jnp.abs(q)
        sub = lax.broadcasted_iota(I32, (8, L), 0)
        for g in range(D // L):
            kq_v[D + g * L:D + g * L + 64, tok] = q[g * L:g * L + 64]
            yield
            kq_v[D + g * L + 64:D + (g + 1) * L, tok] = q[g * L + 64:(g + 1) * L]
            m = [jnp.maximum(a[DH * j:DH * j + 8], a[DH * j + 8:DH * j + 16]) for j in range(8 * g, 8 * g + 8)]
            for w in (4, 2, 1):
                m = [jnp.where((sub & w) == 0,
                               jnp.maximum(m[j], pltpu.roll(m[j], 8 - w, 0)),
                               jnp.maximum(m[j + w], pltpu.roll(m[j + w], w, 0))) for j in range(w)]
            amax = jnp.maximum(m[0], TINY)
            top[0] = jnp.maximum(top[0], amax)
            yield
            qscale_v[H + 8 * g:H + 8 * g + 8, tok] = QMAX / amax
            qscale_v[8 * g:8 * g + 8, tok] = amax * (1.0 / (QMAX * KMAX))

    def v_steps(t):
        vt = project(2, t)
        for r in range(0, D, 64):
            vt_v[t, r // 2:r // 2 + 32, :] = _pack(vt[r:r + 64])
            yield

    def limbs(hd, p):
        r = slice(hd * DH, (hd + 1) * DH)
        tok = _ds(p * TP, TP)
        y = (kq_v[r, tok] - _cat([kstat_v[0, r]] * 2, 1)) * _cat([kstat_v[1, r]] * 2, 1)
        z = _fixed(y, FRAC, 2.0 ** (FRAC - 1))
        b1 = lax.bitcast_convert_type(y * (-1.0 / 3.0) - MAGIC, I32)
        b3 = ((z >> FRAC) - b1 - b1).astype(I16)
        b1 = b1.astype(I16)
        be = (z & (2 ** FRAC - 1)).astype(I16)
        bc = _fixed(y, -FRAC).astype(I16)
        kl = _cat([b1, b1, b1, b1, b3, b3, be, bc], 0).T.astype(I8)
        for j in range(TP // 32):
            limb_v[hd, _ds(p * TP + (j // 4) * L + (3 - j % 4) * 32, 32), :] = kl[32 * j:32 * j + 32]
        x = kq_v[D + hd * DH:D + (hd + 1) * DH, tok] * qscale_v[H + hd:H + hd + 1, tok]
        z = _fixed(x, FRAC, 2.0 ** (FRAC - 1))
        a1 = _fixed(x, -1)
        a2 = (z >> FRAC) - a1
        ac = _fixed(x, -FRAC)
        ae = (z & (2 ** FRAC - 1)) - 2 ** (FRAC - 1)
        ql = _cat([a1, a2, ac, ae], 0).astype(I8)
        for i in range(2):
            limb_v[hd, _ds(S + p * L + 64 * i, 64), :] = ql[:, i * L:(i + 1) * L]

    def phase2(p, top, last=False):
        top = [top]
        gens = [] if last else [q_steps(2 * p + 2 + j, top) for j in range(2)]
        gens += [v_steps(2 * p + j) for j in range(2)]
        lead = done = 6
        for hd in range(lead):
            limbs(hd, p)
        step = 0
        for gen in gens:
            for _ in gen:
                step += 1
                upto = min(H, lead + ((H - lead) * step) // (8 * len(gens) - lead))
                for hd in range(done, upto):
                    limbs(hd, p)
                done = upto
        return top[0]

    top = [jnp.zeros((8, L), F32)]
    for t in range(2):
        for _ in q_steps(t, top):
            pass

    def three_pairs(i, top):
        for u in range(3):
            top = phase2(3 * i + u, top)
        return top

    top = lax.fori_loop(0, (NP - 2) // 3, three_pairs, top[0])
    wait("rest")
    top = phase2(NP - 1, phase2(NP - 2, top), last=True)
    too_wide = jnp.max(jnp.where(top <= TERM_LIMIT, 0.0, 1.0))
    mod_v[...] = _dot(silu_c, wmod_v[:, 2 * D:6 * D])[0:8]
    p_v[...] = jnp.zeros(p_v.shape, p_v.dtype)
    acc_v[...] = jnp.ones(acc_v.shape, acc_v.dtype)

    TQ, HU, G = 4 * L, 8, 2
    NI = (S // TQ) * (H // HU)

    def prepare_weights(i):
        for q in range(-(-(FH + FR) // (16 * NI))):
            r = jnp.minimum((q * NI + i) * 16, FH + FR - 16)
            r1 = jnp.where(r < FH, r, r + FH)
            r2 = jnp.where(r < FH, r + FH, r + FH + FR)
            for w in range(2):
                a1, a2 = wf_v[w, _ds(r1, 16), :].astype(F32), wf_v[w, _ds(r2, 16), :].astype(F32)
                for n, op in enumerate(_lhs7(a1[:, :HD], a1[:, HD:], a2[:, :HD], a2[:, HD:])):
                    for j in range(HD // L):
                        wgu7_v[w, n, j, _ds(r, 16), :] = op[:, j * L:(j + 1) * L].astype(BF16)

    def pv(hd, c, p):
        return _dot(_unpack(vt_v[c, _ds(hd * (DH // 2), DH // 2), :]), p)

    def store_o(o, hd, qb):
        for j in range(TQ // L):
            ot_v[qb * (TQ // L) + j, _ds(hd * (DH // 2), DH // 2), :] = _pack(o[:, j * L:(j + 1) * L])

    def finalize(acc, den, hd, qb, bad):
        l = jnp.sum(den, axis=0, keepdims=True)
        store_o(acc * pltpu.reciprocal(l, full_range=False), hd, qb)
        return jnp.where((l >= DEN_LO) & (l <= DEN_HI), bad, 1.0)

    def attend(i, bad):
        h0, qb = (i % (H // HU)) * HU, i // (H // HU)
        ip = jnp.maximum(i - 1, 0)
        scales = qscale_v[_ds(h0, HU), _ds(qb * TQ, TQ)]
        prev = ((ip % (H // HU)) * HU + HU - 1, ip // (H // HU), NT - G, [_unpack(p_v[a]) for a in range(G)])
        acc, den = acc_v[0:DH], acc_v[DH:DH + 8]
        for u in range(HU):
            ql = _cat([limb_v[h0 + u, _ds(S + qb * (TQ // 2) + 64 * j, 64), :] for j in range(TQ // L)], 1)
            ql = _cat([ql[0:32], ql[0:32], ql], 0)
            scale = jnp.broadcast_to(scales[u:u + 1], (8, TQ))
            d = None
            for c in range(0, NT, G):
                s = jnp.dot(limb_v[h0 + u, c * L:(c + G) * L, :], ql, preferred_element_type=I32)
                e = []
                for j in range(G * L // 8):
                    e.append(jnp.exp2(s[8 * j:8 * j + 8].astype(F32) * scale))
                    d = e[-1] if d is None else d + e[-1]
                p = [_cat([e[16 * a + 4 * (3 - j // 4) + j % 4] for j in range(16)], 0).astype(BF16)
                     for a in range(G)]
                hd, pqb, pc, pp = prev
                o = pv(hd, pc, pp[0]) + pv(hd, pc + 1, pp[1])
                acc = o if acc is None else acc + o
                if pc == NT - G:
                    bad = finalize(acc, den, hd, pqb, bad)
                    acc = None
                prev = (h0 + u, qb, c, p)
            den = d
        for a in range(G):
            p_v[a] = _pack(prev[3][a])
        acc_v[0:DH], acc_v[DH:DH + 8] = acc, den
        prepare_weights(i)
        return bad

    bad = lax.fori_loop(0, jnp.where(too_wide == 0.0, NI, 0), attend, jnp.zeros((1, TQ), F32))
    acc = acc_v[0:DH] + pv(H - 1, NT - 2, _unpack(p_v[0])) + pv(H - 1, NT - 1, _unpack(p_v[1]))
    bad = finalize(acc, acc_v[DH:DH + 8], H - 1, S // TQ - 1, bad)

    @pl.when(jnp.maximum(jnp.max(bad), too_wide) != 0.0)
    def _plain_attention():
        def setup(t, carry):
            k = _dot(h_v[_ds(t * L, L), :], wqkv_v[:, D:2 * D])
            for g in range(D // L):
                kb_v[g, _ds(t * L, L), :] = k[:, g * L:(g + 1) * L].astype(BF16)
            kq_v[D:2 * D, _ds(t * L, L)] = project(0, t)
            return carry

        def weights(i, carry):
            prepare_weights(i)
            return carry

        lax.fori_loop(0, NT, setup, 0)
        lax.fori_loop(0, NI, weights, 0)
        items = (S // TQ) * H
        head = lax.broadcasted_iota(I32, (L, TQ), 0) // DH

        def step(n, cur, nxt, row_max):
            nn = jnp.minimum(n + 1, items - 1)
            g = (nn % H) // (L // DH)
            q = kq_v[_ds(D + g * L, L), _ds((nn // H) * TQ, TQ)]
            q = jnp.where(head == nn % (L // DH), q, 0.0).astype(BF16)
            mx = acc = den = None
            for c in range(NT):
                s = _dot(kb_v[g, c * L:(c + 1) * L, :], q)
                nxt[c * L:(c + 1) * L, :] = s
                t = jnp.max(s.reshape(L // 8, 8, TQ), axis=0)
                mx = t if mx is None else jnp.maximum(mx, t)
                if cur is not None:
                    e = jnp.exp2((cur[c * L:(c + 1) * L, :] - row_max) * logit_scale)
                    t = jnp.sum(e.reshape(L // 8, 8, TQ), axis=0)
                    o = pv(n % H, c, e.astype(BF16))
                    den, acc = (t, o) if c == 0 else (den + t, acc + o)
            if cur is not None:
                store_o(acc / jnp.sum(den, axis=0, keepdims=True), n % H, n // H)
            return jnp.max(mx, axis=0, keepdims=True)

        def two_steps(i, row_max):
            return step(2 * i + 1, sb_v, sa_v, step(2 * i, sa_v, sb_v, row_max))

        lax.fori_loop(0, items // 2, two_steps, step(-1, None, sa_v, None))

    ga, sb, cb1 = mod_v[0:1, 0:D], mod_v[0:1, D:2 * D], 1.0 + mod_v[0:1, 2 * D:3 * D]
    NR = 32

    def norm2(p, r0):
        h1, h2 = [_normalize(x1_v[_ds((2 * p + e) * L + r0, NR), :]) * cb1 + sb for e in range(2)]
        for n, op in enumerate(_rhs7(h1[:, :HD], h2[:, :HD], h1[:, HD:], h2[:, HD:])):
            for j in range(HD // L):
                h7_v[n, j, _ds(p * L + r0, NR), :] = op[:, j * L:(j + 1) * L].astype(BF16)

    def uneven(a, b):
        return jnp.where((a <= BALANCE * b) & (b <= BALANCE * a), 0.0, 1.0)

    def check_rows(w, r1, r2, flag):
        norms = []
        for e, r in enumerate((r1, r2)):
            a = wf_v[w, _ds(r, 16), :].astype(F32)
            a = a * a
            colsq_v[2 * w + e] += a[0:8] + a[8:16]
            norms.append(jnp.sum(a, axis=1, keepdims=True))
        return jnp.maximum(flag, uneven(*norms))

    colsq_v[...] = jnp.zeros(colsq_v.shape, F32)
    row_flag = jnp.zeros((16, 1), F32)
    for p in range(NP):
        rows = slice(p * TP, (p + 1) * TP)
        o = _unpack(_cat([ot_v[2 * p], ot_v[2 * p + 1]], 1)).T
        x1_v[rows, :] = x_v[rows, :].astype(F32) + ga * _dot(o, wo_v[...])
        if p == 1:
            for r0 in range(0, L, NR):
                norm2(0, r0)
        if p == 0:
            for w in range(2):
                for r in range(2 * FH, 2 * FH + FR, 16):
                    row_flag = check_rows(w, r, r + FR, row_flag)
        k = (p - 2) * L
        if 0 <= k < FH:
            for c0 in range(0, HD, L):
                w = [wf_v[2, r + k:r + k + L, c + c0:c + c0 + L].astype(F32) for c in (0, HD) for r in (0, FH)]
                for n, op in enumerate(_lhs7(*w)):
                    wd7_v[n, c0 // 2:(c0 + L) // 2, k:k + L] = _pack(op.astype(BF16).T)
    yt_v[...] = jnp.zeros(yt_v.shape, yt_v.dtype)

    chunks = [(FH, FH + FR)] + [(f, f + L) for f in range(0, FH, L)]

    def out_copy(p):
        rows = _ds(p * TP, TP)
        return pltpu.make_async_copy(out_v.at[rows], out_hbm.at[rows], out_sem)

    def finish(p):
        rows = _ds(p * TP, TP)
        y = _unpack(yt_v[...]).T.astype(F32)
        out_v[rows, :] = (x1_v[rows, :] + mod_v[0:1, 3 * D:4 * D] * y).astype(out_v.dtype)

    def ffn(p, row_flag):
        h7 = [_cat([h7_v[n, j, _ds(p * L, L), :] for j in range(HD // L)], 1) for n in range(7)]
        wd_rest = wf_v[2, 2 * FH:F, :].T
        finish(jnp.maximum(p - 1, 0))
        act7, flag = [], [row_flag]
        for k, (f0, f1) in enumerate(chunks):
            def gate_up(n):
                lhs = _cat([_cat([wgu7_v[w, n, j, f0:f1, :] for j in range(HD // L)], 1) for w in range(2)], 0)
                m = _dot_nt(lhs, h7[n])
                if (k, n) == (1, 6):
                    out_v[_ds(S + 16 * (p % 2), 16), 0:L] = m[-16:].astype(BF16)
                if k and n in (0, 6, 1):
                    w, r = (0, 6, 1).index(n), p * (FH // NP) + (k - 1) * 16
                    wf_v[w, _ds(F + 16 * (p % 2), 16), 0:L] = m[0:16].astype(BF16)
                    flag[0] = check_rows(w, r, FH + r, flag[0])
                return m
            act = [_gelu(c[:f1 - f0]) * c[f1 - f0:] for c in _strassen(gate_up)]
            if f0 < FH:
                act7.append(_rhs7(*act))
            else:
                rest = _cat([_cat(act[:2], 1), _cat(act[2:], 1)], 0).astype(BF16)
        y = _cat([_dot(wd_rest[:HD], rest), _dot(wd_rest[HD:], rest)], 0)
        todo = list(range(0, L, NR))

        def down(n):
            m = _dot(_unpack(wd7_v[n]), _cat([a[n] for a in act7], 0).astype(BF16))
            if todo:
                x1_v[_ds(S + 8 * (p % 2), 8), 0:L] = m[0:8]
                norm2(jnp.minimum(p + 1, NP - 1), todo.pop(0))
            return m
        blk = _strassen(down)
        yt_v[...] = _pack(y + _cat([_cat(blk[:2], 1), _cat(blk[2:], 1)], 0))

        @pl.when(p > 0)
        def _():
            out_copy(p - 1).start()
        return flag[0]

    row_flag = lax.fori_loop(0, NP, ffn, row_flag)
    finish(NP - 1)
    out_copy(NP - 1).start()
    col_flag = jnp.zeros((1, HD), F32)
    for w in range(3):
        t = [jnp.sum(colsq_v[2 * w + e], axis=0, keepdims=True) for e in range(2)]
        t = [t[0][:, :HD], t[0][:, HD:], t[1][:, :HD], t[1][:, HD:]]
        col_flag = jnp.maximum(col_flag, uneven(functools.reduce(jnp.maximum, t), functools.reduce(jnp.minimum, t)))
    redo = jnp.maximum(jnp.max(row_flag), jnp.max(col_flag)) != 0.0
    for p in range(NP):
        out_copy(p).wait()

    @pl.when(redo)
    def _plain_ffn():
        def body(p, carry):
            rows = _ds(p * TP, TP)
            h = (_normalize(x1_v[rows, :]) * cb1 + sb).astype(BF16)
            act = _gelu(_dot_nt(h, wf_v[0, 0:F, :])) * _dot_nt(h, wf_v[1, 0:F, :])
            y = _dot(act.astype(BF16), wf_v[2, 0:F, :])
            out_v[rows, :] = (x1_v[rows, :] + mod_v[0:1, 3 * D:4 * D] * y).astype(out_v.dtype)
            out_copy(p).start()
            return carry
        lax.fori_loop(0, NP, body, 0)
        for p in range(NP):
            out_copy(p).wait()


@jax.jit
def pallas_adaLN_cond__mha_block__geglu_ffn__prompt_kernel(
    A_x: jax.Array,
    A_wqkv: jax.Array,
    A_wo: jax.Array,
    B_x: jax.Array,
    B_w_gate: jax.Array,
    B_w_up: jax.Array,
    B_w_down: jax.Array,
    c: jax.Array,
    w_mod: jax.Array,
):
    del B_x
    B, S, D = A_x.shape
    F = B_w_gate.shape[1]
    assert (B, S, D, F) == (1, 2048, 512, 1376), "tiling is laid out for these shapes"
    vmem = pltpu.VMEM
    scratch = [
        vmem((S, D), BF16),
        vmem((D, 3 * D), BF16),
        vmem((D, D), BF16),
        vmem((3, F + 32, D), BF16),
        vmem((1, D), BF16),
        vmem((D, 6 * D), BF16),
        vmem((S + 32, D), BF16),
        vmem((8, 4 * D), F32),
        vmem((3, D // 2, D), I32),
        vmem((S, D), BF16),
        vmem((2 * D, S), F32),
        vmem((3, D, L), F32),
        vmem((2 * H, S), F32),
        vmem((H, S + S // 2, L), I8),
        vmem((S // L, D // 2, L), I32),
        vmem((2, L // 2, 4 * L), I32),
        vmem((D // H + 8, 4 * L), F32),
        vmem((S // L, D // 2, L), I32),
        vmem((D // L, S, L), BF16),
        vmem((S, 4 * L), F32),
        vmem((S, 4 * L), F32),
        vmem((2, 7, 2, F // 2, L), BF16),
        vmem((7, D // 4, F // (2 * L) * L), I32),
        vmem((S + 16, D), F32),
        vmem((7, 2, S // 2, L), BF16),
        vmem((D // 2, 2 * L), I32),
        vmem((6, 8, D), F32),
        pltpu.SemaphoreType.DMA((3 + len(X_PIECES),)),
        pltpu.SemaphoreType.DMA(()),
    ]
    out = pl.pallas_call(
        _block_kernel,
        out_shape=jax.ShapeDtypeStruct((S, D), A_x.dtype),
        in_specs=[pl.BlockSpec(memory_space=pltpu.HBM)] * 8,
        out_specs=pl.BlockSpec(memory_space=pltpu.HBM),
        scratch_shapes=scratch,
        compiler_params=pltpu.CompilerParams(vmem_limit_bytes=100 * 2 ** 20),
        name="adaln_mha_geglu_blk",
    )(A_x.reshape(S, D), A_wqkv, A_wo, B_w_gate.T, B_w_up.T, B_w_down, c, w_mod)
    return out.reshape(B, S, D)
```

```python
import functools
import math

import jax
import jax.numpy as jnp
from jax import lax
import jax.experimental.pallas as pl
import jax.experimental.pallas.tpu as pltpu

F32, BF16, I32, I16, I8 = jnp.float32, jnp.bfloat16, jnp.int32, jnp.int16, jnp.int8

H = 32
L = 128
LN_EPS = 1e-5

MAGIC = 1.5 * 2.0 ** 23
QMAX, KMAX = 253.0, 376.0
FRAC = 4
TINY = 1e-30
TERM_LIMIT = 24.0
DEN_LO, DEN_HI = 2.0 ** -40, 2.0 ** 40
BALANCE = 4.0

X_PIECES = ((2, 1), (4, 3), (10, 9), (16, 16))


def _dot(a, b):
    return jnp.dot(a, b, preferred_element_type=F32)


def _dot_nt(a, b):
    return lax.dot_general(a, b, (((1,), (1,)), ((), ())), preferred_element_type=F32)


def _cat(parts, axis):
    return jnp.concatenate(parts, axis=axis)


def _ds(start, size):
    return pl.ds(start if isinstance(start, int) else pl.multiple_of(start, size), size)


def _pack(v):
    return pltpu.bitcast(v.astype(BF16), I32)


def _unpack(v):
    return pltpu.bitcast(v, BF16)


def _normalize(x):
    xc = x - jnp.mean(x, axis=-1, keepdims=True)
    return xc * lax.rsqrt(jnp.mean(xc * xc, axis=-1, keepdims=True) + LN_EPS)


def _gelu(x):
    c0 = math.sqrt(2.0 / math.pi)
    return (0.5 * x) * (1.0 + jnp.tanh(x * (c0 + (c0 * 0.044715) * (x * x))))


def _fixed(v, shift, bias=0.0):
    return lax.bitcast_convert_type(v + (MAGIC + bias) * 2.0 ** -shift, I32)


def _lhs7(a11, a12, a21, a22):
    return [a11 + a22, a21 + a22, a11, a22, a11 + a12, a21 - a11, a12 - a22]


def _rhs7(b11, b12, b21, b22):
    return [b11 + b22, b11, b12 - b22, b21 - b11, b22, b11 + b12, b21 + b22]


def _strassen(prod):
    c11 = c22 = prod(0)
    c22 = c22 + prod(5)
    c11 = c11 + prod(6)
    m = prod(1)
    c21, c22 = m, c22 - m
    m = prod(3)
    c21, c11 = c21 + m, c11 + m
    m = prod(2)
    c12, c22 = m, c22 + m
    m = prod(4)
    c12, c11 = c12 + m, c11 - m
    return c11, c12, c21, c22


def _block_kernel(x_hbm, wqkv_hbm, wo_hbm, wg_hbm, wu_hbm, wd_hbm, c_hbm, wmod_hbm, out_hbm,
                  x_v, wqkv_v, wo_v, wf_v, c_v, wmod_v, out_v,
                  mod_v, wt_v, h_v, kq_v, kstat_v, qscale_v, limb_v, vt_v, p_v, acc_v, ot_v,
                  kb_v, sa_v, sb_v, wgu7_v, wd7_v, x1_v, h7_v, yt_v, colsq_v, sem, out_sem):
    S, D = x_v.shape
    F = wd_hbm.shape[0]
    DH, HD = D // H, D // 2
    FH = (F // (2 * L)) * L
    FR = (F - 2 * FH) // 2
    TP = 2 * L
    NT, NP = S // L, S // TP
    logit_scale = DH ** -0.5 * math.log2(math.e)

    def cols(a, b):
        return (slice(None), slice(a * D, b * D))

    x_rows = [slice(a * L, b * L) for a, (b, _) in zip([0] + [n for n, _ in X_PIECES], X_PIECES)]
    last_x = "x%d" % (len(x_rows) - 1)
    groups = {"wk": [(c_hbm, c_v), (wqkv_hbm.at[cols(1, 2)], wqkv_v.at[cols(1, 2)])],
              "x0": [(x_hbm.at[x_rows[0]], x_v.at[x_rows[0]])],
              "mod": [(wmod_hbm.at[cols(0, 2)], wmod_v.at[cols(0, 2)])]}
    for i in range(1, len(x_rows)):
        groups["x%d" % i] = [(x_hbm.at[x_rows[i]], x_v.at[x_rows[i]])]
    groups[last_x] += [(wqkv_hbm.at[cols(w, w + 1)], wqkv_v.at[cols(w, w + 1)]) for w in (0, 2)]
    groups["rest"] = [(wmod_hbm.at[cols(2, 6)], wmod_v.at[cols(2, 6)]), (wo_hbm, wo_v)]
    groups["rest"] += [(src, wf_v.at[w, 0:F]) for w, src in enumerate((wg_hbm, wu_hbm, wd_hbm))]
    dma = {name: [pltpu.make_async_copy(src, dst, sem.at[i]) for src, dst in group]
           for i, (name, group) in enumerate(groups.items())}
    for group in dma.values():
        for copy in group:
            copy.start()

    def wait(name):
        for copy in dma[name]:
            copy.wait()

    def transpose_weight(w):
        wt_v[w] = _pack(wqkv_v[:, w * D:(w + 1) * D].T)

    def project(w, t):
        return _dot_nt(_unpack(wt_v[w]), h_v[_ds(t * L, L), :])

    wait("wk")
    cv = c_v[...].astype(F32)
    silu_c = jnp.broadcast_to(cv * jax.nn.sigmoid(cv), (16, D)).astype(BF16)
    transpose_weight(1)
    wait("x0")
    xn = _normalize(x_v[x_rows[0], :].astype(F32))
    wait("mod")
    mod_a = _dot(silu_c, wmod_v[:, 0:2 * D])
    sa, ca1 = mod_a[0:1, 0:D], 1.0 + mod_a[0:1, D:2 * D]

    hi = lo = None
    n0 = k0 = 0
    for i, (n1, k1) in enumerate(X_PIECES):
        if i:
            wait("x%d" % i)
        for t in range(n0, n1):
            rows = slice(t * L, (t + 1) * L)
            xt = _normalize(x_v[rows, :].astype(F32)) if i else xn[rows]
            h_v[rows, :] = (xt * ca1 + sa).astype(BF16)
        for t in range(k0, k1):
            kt = project(1, t)
            kq_v[0:D, t * L:(t + 1) * L] = kt
            hi = kt if hi is None else jnp.maximum(hi, kt)
            lo = kt if lo is None else jnp.minimum(lo, kt)
        n0, k0 = n1, k1
    transpose_weight(0)
    transpose_weight(2)
    hi = jnp.max(hi, axis=1, keepdims=True)
    lo = jnp.min(lo, axis=1, keepdims=True)
    mid = 0.5 * hi + 0.5 * lo
    rad = jnp.maximum(jnp.maximum(hi - mid, mid - lo), TINY)
    kstat_v[0] = jnp.broadcast_to(mid, (D, L))
    kstat_v[1] = jnp.broadcast_to(KMAX / rad, (D, L))
    kstat_v[2] = jnp.broadcast_to(rad * logit_scale, (D, L))

    def q_steps(t, top):
        tok = _ds(t * L, L)
        q = project(0, t) * kstat_v[2]
        a = jnp.abs(q)
        sub = lax.broadcasted_iota(I32, (8, L), 0)
        for g in range(D // L):
            kq_v[D + g * L:D + g * L + 64, tok] = q[g * L:g * L + 64]
            yield
            kq_v[D + g * L + 64:D + (g + 1) * L, tok] = q[g * L + 64:(g + 1) * L]
            m = [jnp.maximum(a[DH * j:DH * j + 8], a[DH * j + 8:DH * j + 16]) for j in range(8 * g, 8 * g + 8)]
            for w in (4, 2, 1):
                m = [jnp.where((sub & w) == 0,
                               jnp.maximum(m[j], pltpu.roll(m[j], 8 - w, 0)),
                               jnp.maximum(m[j + w], pltpu.roll(m[j + w], w, 0))) for j in range(w)]
            amax = jnp.maximum(m[0], TINY)
            top[0] = jnp.maximum(top[0], amax)
            yield
            qscale_v[H + 8 * g:H + 8 * g + 8, tok] = QMAX / amax
            qscale_v[8 * g:8 * g + 8, tok] = amax * (1.0 / (QMAX * KMAX))

    def v_steps(t):
        vt = project(2, t)
        for r in range(0, D, 64):
            vt_v[t, r // 2:r // 2 + 32, :] = _pack(vt[r:r + 64])
            yield

    def limbs(hd, p):
        r = slice(hd * DH, (hd + 1) * DH)
        tok = _ds(p * TP, TP)
        y = (kq_v[r, tok] - _cat([kstat_v[0, r]] * 2, 1)) * _cat([kstat_v[1, r]] * 2, 1)
        z = _fixed(y, FRAC, 2.0 ** (FRAC - 1))
        b1 = lax.bitcast_convert_type(y * (-1.0 / 3.0) - MAGIC, I32)
        b3 = ((z >> FRAC) - b1 - b1).astype(I16)
        b1 = b1.astype(I16)
        be = (z & (2 ** FRAC - 1)).astype(I16)
        bc = _fixed(y, -FRAC).astype(I16)
        kl = _cat([b1, b1, b1, b1, b3, b3, be, bc], 0).T.astype(I8)
        for j in range(TP // 32):
            limb_v[hd, _ds(p * TP + (j // 4) * L + (3 - j % 4) * 32, 32), :] = kl[32 * j:32 * j + 32]
        x = kq_v[D + hd * DH:D + (hd + 1) * DH, tok] * qscale_v[H + hd:H + hd + 1, tok]
        z = _fixed(x, FRAC, 2.0 ** (FRAC - 1))
        a1 = _fixed(x, -1)
        a2 = (z >> FRAC) - a1
        ac = _fixed(x, -FRAC)
        ae = (z & (2 ** FRAC - 1)) - 2 ** (FRAC - 1)
        ql = _cat([a1, a2, ac, ae], 0).astype(I8)
        for i in range(2):
            limb_v[hd, _ds(S + p * L + 64 * i, 64), :] = ql[:, i * L:(i + 1) * L]

    def phase2(p, top, last=False):
        top = [top]
        gens = [] if last else [q_steps(2 * p + 2 + j, top) for j in range(2)]
        gens += [v_steps(2 * p + j) for j in range(2)]
        lead = done = 6
        for hd in range(lead):
            limbs(hd, p)
        step = 0
        for gen in gens:
            for _ in gen:
                step += 1
                upto = min(H, lead + ((H - lead) * step) // (8 * len(gens) - lead))
                for hd in range(done, upto):
                    limbs(hd, p)
                done = upto
        return top[0]

    top = [jnp.zeros((8, L), F32)]
    for t in range(2):
        for _ in q_steps(t, top):
            pass

    def three_pairs(_, carry):
        p, top = carry
        for u in range(3):
            top = phase2(p + u, top)
        return p + 3, top

    p, top = lax.fori_loop(0, (NP - 2) // 3, three_pairs, (0, top[0]))
    wait("rest")
    top = phase2(p + 1, phase2(p, top), last=True)
    too_wide = jnp.max(jnp.where(top <= TERM_LIMIT, 0.0, 1.0))
    mod_v[...] = _dot(silu_c, wmod_v[:, 2 * D:6 * D])[0:8]
    p_v[...] = jnp.zeros(p_v.shape, p_v.dtype)
    acc_v[...] = jnp.ones(acc_v.shape, acc_v.dtype)

    TQ, HU, G = 4 * L, 8, 2
    NI = (S // TQ) * (H // HU)

    def prepare_weights(i):
        per = -(-(FH + FR) // (16 * NI))
        for q in range(per):
            r = jnp.minimum((per * i + q) * 16, FH + FR - 16)
            r1 = jnp.where(r < FH, r, r + FH)
            r2 = jnp.where(r < FH, r + FH, r + FH + FR)
            for w in range(2):
                a1, a2 = wf_v[w, _ds(r1, 16), :].astype(F32), wf_v[w, _ds(r2, 16), :].astype(F32)
                for n, op in enumerate(_lhs7(a1[:, :HD], a1[:, HD:], a2[:, :HD], a2[:, HD:])):
                    for j in range(HD // L):
                        wgu7_v[w, n, j, _ds(r, 16), :] = op[:, j * L:(j + 1) * L].astype(BF16)

    def pv(hd, c, p):
        return _dot(_unpack(vt_v[c, _ds(hd * (DH // 2), DH // 2), :]), p)

    def store_o(o, hd, qb):
        for j in range(TQ // L):
            ot_v[qb * (TQ // L) + j, _ds(hd * (DH // 2), DH // 2), :] = _pack(o[:, j * L:(j + 1) * L])

    def finalize(acc, den, hd, qb, bad):
        l = jnp.sum(den, axis=0, keepdims=True)
        store_o(acc * pltpu.reciprocal(l, full_range=False), hd, qb)
        return jnp.where((l >= DEN_LO) & (l <= DEN_HI), bad, 1.0)

    def attend(i, bad):
        h0, qb = (i % (H // HU)) * HU, i // (H // HU)
        ip = jnp.maximum(i - 1, 0)
        scales = qscale_v[_ds(h0, HU), _ds(qb * TQ, TQ)]
        prev = ((ip % (H // HU)) * HU + HU - 1, ip // (H // HU), NT - G, [_unpack(p_v[a]) for a in range(G)])
        acc, den = acc_v[0:DH], acc_v[DH:DH + 8]
        for u in range(HU):
            ql = _cat([limb_v[h0 + u, _ds(S + qb * (TQ // 2) + 64 * j, 64), :] for j in range(TQ // L)], 1)
            ql = _cat([ql[0:32], ql[0:32], ql], 0)
            scale = jnp.broadcast_to(scales[u:u + 1], (8, TQ))
            d = None
            for c in range(0, NT, G):
                s = jnp.dot(limb_v[h0 + u, c * L:(c + G) * L, :], ql, preferred_element_type=I32)
                e = []
                for j in range(G * L // 8):
                    e.append(jnp.exp2(s[8 * j:8 * j + 8].astype(F32) * scale))
                    d = e[-1] if d is None else d + e[-1]
                p = [_cat([e[16 * a + 4 * (3 - j // 4) + j % 4] for j in range(16)], 0).astype(BF16)
                     for a in range(G)]
                hd, pqb, pc, pp = prev
                o = pv(hd, pc, pp[0]) + pv(hd, pc + 1, pp[1])
                acc = o if acc is None else acc + o
                if pc == NT - G:
                    bad = finalize(acc, den, hd, pqb, bad)
                    acc = None
                prev = (h0 + u, qb, c, p)
            den = d
        for a in range(G):
            p_v[a] = _pack(prev[3][a])
        acc_v[0:DH], acc_v[DH:DH + 8] = acc, den
        prepare_weights(i)
        return bad

    bad = lax.fori_loop(0, jnp.where(too_wide == 0.0, NI, 0), attend, jnp.zeros((1, TQ), F32))
    acc = acc_v[0:DH] + pv(H - 1, NT - 2, _unpack(p_v[0])) + pv(H - 1, NT - 1, _unpack(p_v[1]))
    bad = finalize(acc, acc_v[DH:DH + 8], H - 1, S // TQ - 1, bad)

    @pl.when(jnp.maximum(jnp.max(bad), too_wide) != 0.0)
    def _plain_attention():
        def setup(t, carry):
            k = _dot(h_v[_ds(t * L, L), :], wqkv_v[:, D:2 * D])
            for g in range(D // L):
                kb_v[g, _ds(t * L, L), :] = k[:, g * L:(g + 1) * L].astype(BF16)
            kq_v[D:2 * D, _ds(t * L, L)] = project(0, t)
            return carry

        def weights(i, carry):
            prepare_weights(i)
            return carry

        lax.fori_loop(0, NT, setup, 0)
        lax.fori_loop(0, NI, weights, 0)
        items = (S // TQ) * H
        head = lax.broadcasted_iota(I32, (L, TQ), 0) // DH

        def step(n, cur, nxt, row_max):
            nn = jnp.minimum(n + 1, items - 1)
            g = (nn % H) // (L // DH)
            q = kq_v[_ds(D + g * L, L), _ds((nn // H) * TQ, TQ)]
            q = jnp.where(head == nn % (L // DH), q, 0.0).astype(BF16)
            mx = acc = den = None
            for c in range(NT):
                s = _dot(kb_v[g, c * L:(c + 1) * L, :], q)
                nxt[c * L:(c + 1) * L, :] = s
                t = jnp.max(s.reshape(L // 8, 8, TQ), axis=0)
                mx = t if mx is None else jnp.maximum(mx, t)
                if cur is not None:
                    e = jnp.exp2((cur[c * L:(c + 1) * L, :] - row_max) * logit_scale)
                    t = jnp.sum(e.reshape(L // 8, 8, TQ), axis=0)
                    o = pv(n % H, c, e.astype(BF16))
                    den, acc = (t, o) if c == 0 else (den + t, acc + o)
            if cur is not None:
                store_o(acc / jnp.sum(den, axis=0, keepdims=True), n % H, n // H)
            return jnp.max(mx, axis=0, keepdims=True)

        def two_steps(i, row_max):
            return step(2 * i + 1, sb_v, sa_v, step(2 * i, sa_v, sb_v, row_max))

        lax.fori_loop(0, items // 2, two_steps, step(-1, None, sa_v, None))

    ga, sb, cb1 = mod_v[0:1, 0:D], mod_v[0:1, D:2 * D], 1.0 + mod_v[0:1, 2 * D:3 * D]
    NR = 32

    def norm2(p, r0):
        h1, h2 = [_normalize(x1_v[_ds((2 * p + e) * L + r0, NR), :]) * cb1 + sb for e in range(2)]
        for n, op in enumerate(_rhs7(h1[:, :HD], h2[:, :HD], h1[:, HD:], h2[:, HD:])):
            for j in range(HD // L):
                h7_v[n, j, _ds(p * L + r0, NR), :] = op[:, j * L:(j + 1) * L].astype(BF16)

    def uneven(a, b):
        return jnp.where((a <= BALANCE * b) & (b <= BALANCE * a), 0.0, 1.0)

    def check_rows(w, r1, r2, flag):
        norms = []
        for e, r in enumerate((r1, r2)):
            a = wf_v[w, _ds(r, 16), :].astype(F32)
            a = a * a
            colsq_v[2 * w + e] += a[0:8] + a[8:16]
            norms.append(jnp.sum(a, axis=1, keepdims=True))
        return jnp.maximum(flag, uneven(*norms))

    colsq_v[...] = jnp.zeros(colsq_v.shape, F32)
    row_flag = jnp.zeros((16, 1), F32)
    for p in range(NP):
        rows = slice(p * TP, (p + 1) * TP)
        o = _unpack(_cat([ot_v[2 * p], ot_v[2 * p + 1]], 1)).T
        x1_v[rows, :] = x_v[rows, :].astype(F32) + ga * _dot(o, wo_v[...])
        if p == 1:
            for r0 in range(0, L, NR):
                norm2(0, r0)
        if p == 0:
            for w in range(2):
                for r in range(2 * FH, 2 * FH + FR, 16):
                    row_flag = check_rows(w, r, r + FR, row_flag)
        k = (p - 2) * L
        if 0 <= k < FH:
            for c0 in range(0, HD, L):
                w = [wf_v[2, r + k:r + k + L, c + c0:c + c0 + L].astype(F32) for c in (0, HD) for r in (0, FH)]
                for n, op in enumerate(_lhs7(*w)):
                    wd7_v[n, c0 // 2:(c0 + L) // 2, k:k + L] = _pack(op.astype(BF16).T)
    yt_v[...] = jnp.zeros(yt_v.shape, yt_v.dtype)

    chunks = [(FH, FH + FR)] + [(f, f + L) for f in range(0, FH, L)]

    def out_copy(p):
        rows = _ds(p * TP, TP)
        return pltpu.make_async_copy(out_v.at[rows], out_hbm.at[rows], out_sem)

    def finish(p):
        rows = _ds(p * TP, TP)
        y = _unpack(yt_v[...]).T.astype(F32)
        out_v[rows, :] = (x1_v[rows, :] + mod_v[0:1, 3 * D:4 * D] * y).astype(out_v.dtype)

    def ffn(p, row_flag):
        h7 = [_cat([h7_v[n, j, _ds(p * L, L), :] for j in range(HD // L)], 1) for n in range(7)]
        wd_rest = wf_v[2, 2 * FH:F, :].T
        finish(jnp.maximum(p - 1, 0))
        act7, flag = [], [row_flag]
        for k, (f0, f1) in enumerate(chunks):
            def gate_up(n):
                lhs = _cat([_cat([wgu7_v[w, n, j, f0:f1, :] for j in range(HD // L)], 1) for w in range(2)], 0)
                m = _dot_nt(lhs, h7[n])
                if (k, n) == (1, 6):
                    out_v[_ds(S + 16 * (p % 2), 16), 0:L] = m[-16:].astype(BF16)
                if k and n in (0, 6, 1):
                    w, r = (0, 6, 1).index(n), p * (FH // NP) + (k - 1) * 16
                    wf_v[w, _ds(F + 16 * (p % 2), 16), 0:L] = m[0:16].astype(BF16)
                    flag[0] = check_rows(w, r, FH + r, flag[0])
                return m
            act = [_gelu(c[:f1 - f0]) * c[f1 - f0:] for c in _strassen(gate_up)]
            if f0 < FH:
                act7.append(_rhs7(*act))
            else:
                rest = _cat([_cat(act[:2], 1), _cat(act[2:], 1)], 0).astype(BF16)
        y = _cat([_dot(wd_rest[:HD], rest), _dot(wd_rest[HD:], rest)], 0)
        todo = list(range(0, L, NR))

        def down(n):
            m = _dot(_unpack(wd7_v[n]), _cat([a[n] for a in act7], 0).astype(BF16))
            if todo:
                x1_v[_ds(S + 8 * (p % 2), 8), 0:L] = m[0:8]
                norm2(jnp.minimum(p + 1, NP - 1), todo.pop(0))
            return m
        blk = _strassen(down)
        yt_v[...] = _pack(y + _cat([_cat(blk[:2], 1), _cat(blk[2:], 1)], 0))

        @pl.when(p > 0)
        def _():
            out_copy(p - 1).start()
        return flag[0]

    row_flag = lax.fori_loop(0, NP, ffn, row_flag)
    finish(NP - 1)
    out_copy(NP - 1).start()
    col_flag = jnp.zeros((1, HD), F32)
    for w in range(3):
        t = [jnp.sum(colsq_v[2 * w + e], axis=0, keepdims=True) for e in range(2)]
        t = [t[0][:, :HD], t[0][:, HD:], t[1][:, :HD], t[1][:, HD:]]
        col_flag = jnp.maximum(col_flag, uneven(functools.reduce(jnp.maximum, t), functools.reduce(jnp.minimum, t)))
    redo = jnp.maximum(jnp.max(row_flag), jnp.max(col_flag)) != 0.0
    for p in range(NP):
        out_copy(p).wait()

    @pl.when(redo)
    def _plain_ffn():
        def body(p, carry):
            rows = _ds(p * TP, TP)
            h = (_normalize(x1_v[rows, :]) * cb1 + sb).astype(BF16)
            act = _gelu(_dot_nt(h, wf_v[0, 0:F, :])) * _dot_nt(h, wf_v[1, 0:F, :])
            y = _dot(act.astype(BF16), wf_v[2, 0:F, :])
            out_v[rows, :] = (x1_v[rows, :] + mod_v[0:1, 3 * D:4 * D] * y).astype(out_v.dtype)
            out_copy(p).start()
            return carry
        lax.fori_loop(0, NP, body, 0)
        for p in range(NP):
            out_copy(p).wait()


@jax.jit
def pallas_adaLN_cond__mha_block__geglu_ffn__prompt_kernel(
    A_x: jax.Array,
    A_wqkv: jax.Array,
    A_wo: jax.Array,
    B_x: jax.Array,
    B_w_gate: jax.Array,
    B_w_up: jax.Array,
    B_w_down: jax.Array,
    c: jax.Array,
    w_mod: jax.Array,
):
    del B_x
    B, S, D = A_x.shape
    F = B_w_gate.shape[1]
    assert (B, S, D, F) == (1, 2048, 512, 1376), "tiling is laid out for these shapes"
    vmem = pltpu.VMEM
    scratch = [
        vmem((S, D), BF16),
        vmem((D, 3 * D), BF16),
        vmem((D, D), BF16),
        vmem((3, F + 32, D), BF16),
        vmem((1, D), BF16),
        vmem((D, 6 * D), BF16),
        vmem((S + 32, D), BF16),
        vmem((8, 4 * D), F32),
        vmem((3, D // 2, D), I32),
        vmem((S, D), BF16),
        vmem((2 * D, S), F32),
        vmem((3, D, L), F32),
        vmem((2 * H, S), F32),
        vmem((H, S + S // 2, L), I8),
        vmem((S // L, D // 2, L), I32),
        vmem((2, L // 2, 4 * L), I32),
        vmem((D // H + 8, 4 * L), F32),
        vmem((S // L, D // 2, L), I32),
        vmem((D // L, S, L), BF16),
        vmem((S, 4 * L), F32),
        vmem((S, 4 * L), F32),
        vmem((2, 7, 2, F // 2, L), BF16),
        vmem((7, D // 4, F // (2 * L) * L), I32),
        vmem((S + 16, D), F32),
        vmem((7, 2, S // 2, L), BF16),
        vmem((D // 2, 2 * L), I32),
        vmem((6, 8, D), F32),
        pltpu.SemaphoreType.DMA((3 + len(X_PIECES),)),
        pltpu.SemaphoreType.DMA(()),
    ]
    out = pl.pallas_call(
        _block_kernel,
        out_shape=jax.ShapeDtypeStruct((S, D), A_x.dtype),
        in_specs=[pl.BlockSpec(memory_space=pltpu.HBM)] * 8,
        out_specs=pl.BlockSpec(memory_space=pltpu.HBM),
        scratch_shapes=scratch,
        compiler_params=pltpu.CompilerParams(vmem_limit_bytes=100 * 2 ** 20),
        name="adaln_mha_geglu_blk",
    )(A_x.reshape(S, D), A_wqkv, A_wo, B_w_gate.T, B_w_up.T, B_w_down, c, w_mod)
    return out.reshape(B, S, D)
```
